```python
import os as _os
_os.environ.setdefault("JAX_PLATFORMS", "cpu")
import jax
import jax.numpy as jnp

def _softmax(x, axis=-1):
    return jax.nn.softmax(x, axis=axis)
def _gelu(x):
    return jax.nn.gelu(x, approximate=True)
def _silu(x):
    return jax.nn.silu(x)
def _sigmoid(x):
    return jax.nn.sigmoid(x)
def _layernorm(x, axis=-1, eps=1e-5):
    m = jnp.mean(x, axis=axis, keepdims=True)
    v = jnp.var(x, axis=axis, keepdims=True)
    return (x - m) / jnp.sqrt(v + eps)
def _scatter_add(tgt, idx, src, axis=0):
    return tgt.at[idx].add(src)
def _segment_sum(src, seg, n):
    return jax.ops.segment_sum(src, seg, n)
class _Rng:
    def __init__(self, key):
        self._k = key
    def _next(self):
        self._k, sub = jax.random.split(self._k)
        return sub
    def normal(self, shape):
        return jax.random.normal(self._next(), shape, dtype=jnp.bfloat16)
    def randint(self, lo, hi, shape):
        return jax.random.randint(self._next(), shape, lo, hi, dtype=jnp.int32)
    def uniform(self, shape, lo=0.0, hi=1.0):
        return jax.random.uniform(self._next(), shape, jnp.bfloat16, lo, hi)
    def permutation(self, n):
        return jax.random.permutation(self._next(), n)


kernel_name = 'concat_heads__mha_block__linear_attn_block__prompt'

def setup_inputs():
    _rng = _Rng(jax.random.key(int.from_bytes(__import__("os").urandom(4), "little")))
    _w = (lambda a: (lambda t: t.astype(jnp.bfloat16) if jnp.issubdtype(t.dtype, jnp.floating) else t)(jnp.asarray(a)))
    def _A_setup():
        B, S, D, H = 1, 2048, 1024, 32
        return {
            "x": _w((lambda *s: _rng.normal(s) * 0.2)(B, S, D)),
            "wqkv": _w((lambda *s: _rng.normal(s) * 0.2)(D, 3 * D)),
            "wo": _w((lambda *s: _rng.normal(s) * 0.05)(D, D)),
        }
    _A_in = _A_setup()

    def _B_setup():
        B, S, D = 1, 2048, 1024
        return {
            "x": _w((lambda *s: _rng.normal(s) * 0.05)(B, S, D)),
            "wqkv": _w((lambda *s: _rng.normal(s) * 1.6)(D, 3 * D)),
            "wo": _w((lambda *s: _rng.normal(s) * 0.1)(D, D)),
        }
    _B_in = _B_setup()

    return {
        "A_x": _A_in["x"],
        "A_wqkv": _A_in["wqkv"],
        "A_wo": _A_in["wo"],
        "B_x": _B_in["x"],
        "B_wqkv": _B_in["wqkv"],
        "B_wo": _B_in["wo"],
    }

def reference(A_x, A_wqkv, A_wo, B_x, B_wqkv, B_wo):
    def _A_ref(x, wqkv, wo):
        B, S, D = x.shape
        H = 32
        Dh = D // H
        qkv = (lambda x, *d: x.transpose(*d))((x @ wqkv).reshape(B, S, 3, H, Dh), 2, 0, 3, 1, 4)
        q, k, v = qkv[0], qkv[1], qkv[2]
        scores = jnp.einsum("bhqd,bhkd->bhqk", q, k) * (Dh ** -0.5)
        p = _softmax(scores, axis=-1)
        o = jnp.einsum("bhqk,bhkd->bhqd", p, v)
        return (lambda x, *d: x.transpose(*d))(o, 0, 2, 1, 3).reshape(B, S, D) @ wo

    def _B_ref(x, wqkv, wo):
        B, S, D = x.shape
        H = 32; Dh = D // H
        qkv = (lambda x, *d: x.transpose(*d))((x @ wqkv).reshape(B, S, 3, H, Dh), 2, 0, 3, 1, 4)
        q, k, v = qkv[0], qkv[1], qkv[2]
        phi = lambda t: jnp.where(t > 0, t + 1, jnp.exp(t)) + 1e-6
        pq, pk = phi(q), phi(k)
        kv = jnp.einsum("bhsd,bhse->bhde", pk, v)
        z = jnp.einsum("bhsd->bhd", pk)
        num = jnp.einsum("bhqd,bhde->bhqe", pq, kv)
        den = jnp.einsum("bhqd,bhd->bhq", pq, z)[..., None] + 1e-6
        o = num / den
        return (lambda x, *d: x.transpose(*d))(o, 0, 2, 1, 3).reshape(B, S, D) @ wo

    a = _A_ref(A_x, A_wqkv, A_wo)
    b = _B_ref(B_x, B_wqkv, B_wo)
    return jnp.concatenate([a, b], axis=-1)
```

```python
import math

import jax
import jax.numpy as jnp
import jax.experimental.pallas as pl
import jax.experimental.pallas.tpu as pltpu

S = 2048
D = 1024
H = 32
DH = D // H
G = D // 128

TQ = 512
CK = 128
NC = S // CK
NQ = S // TQ
LAG = 3
UNROLL = 4
RB = 512
CB = 512

F32 = jnp.float32
BF16 = jnp.bfloat16
NN = (((1,), (0,)), ((), ()))
NT = (((1,), (1,)), ((), ()))
TN = (((0,), (0,)), ((), ()))


def _dot(a, b, dims=NN):
  return jax.lax.dot_general(a, b, dims, preferred_element_type=F32)


def _phi(t):
  return jnp.where(t > 0, t + 1.0, jnp.exp(t)) + 1e-6


def _kernel(
    xa_hbm, wa_hbm, woa_hbm, xb_hbm, wb_hbm, wob_hbm, out_hbm,
    xa, wa, woa, xb, wb, wob,
    pq, kv, zs, mb, outb,
    qt, kk, vt, s0, s1, m0, m1, ot, outa,
    in_sem, out_sem,
):
  nrb, ncb = S // RB, D // CB

  def rows_copy(src, dst, i, sem):
    return pltpu.make_async_copy(
        src.at[pl.ds(i * RB, RB), :], dst.at[pl.ds(i * RB, RB), :], in_sem.at[sem])

  def cols_copy(src, dst, c, sem):
    return pltpu.make_async_copy(
        src.at[:, pl.ds(c * CB, CB)], dst.at[:, pl.ds(c * CB, CB)], in_sem.at[sem])

  xb_cp = [rows_copy(xb_hbm, xb, i, i) for i in range(nrb)]
  wb_cp = [[cols_copy(wb_hbm, wb, p * ncb + j, nrb + 3 * j + p) for p in range(3)]
           for j in range(ncb)]
  base = nrb + 3 * ncb
  wob_cp = pltpu.make_async_copy(wob_hbm, wob, in_sem.at[base])
  xa_cp = pltpu.make_async_copy(xa_hbm, xa, in_sem.at[base + 1])
  wa_cp = pltpu.make_async_copy(wa_hbm, wa, in_sem.at[base + 2])
  woa_cp = pltpu.make_async_copy(woa_hbm, woa, in_sem.at[base + 3])
  for cp in ([xb_cp[0]] + wb_cp[0] + xb_cp[1:] + wb_cp[1]
             + [wob_cp, xa_cp, wa_cp, woa_cp]):
    cp.start()

  kv[...] = jnp.zeros_like(kv)
  zs[...] = jnp.zeros_like(zs)

  def b_proj(n, carry):
    j, i = n // nrb, n % nrb
    for i_ in range(nrb):
      @pl.when(n == i_)
      def _():
        xb_cp[i_].wait()
    for j_ in range(ncb):
      @pl.when(n == j_ * nrb)
      def _():
        for cp in wb_cp[j_]:
          cp.wait()
    rows = pl.ds(pl.multiple_of(i * RB, RB), RB)
    x = xb[rows, :]

    def cols(p):
      return pl.ds(pl.multiple_of(p * D + j * CB, CB), CB)

    pk = _phi(_dot(x, wb[:, cols(1)])).astype(BF16)
    v = _dot(x, wb[:, cols(2)]).astype(BF16)
    pq[rows, cols(0)] = _phi(_dot(x, wb[:, cols(0)])).astype(BF16)
    zs[j] += jnp.sum(pk.astype(F32).reshape(RB // 8, 8, CB), axis=0)
    for u in range(CB // 128):
      lanes = slice(u * 128, (u + 1) * 128)
      kv[j * (CB // 128) + u] += _dot(pk[:, lanes], v[:, lanes], TN)
    return carry

  jax.lax.fori_loop(0, ncb * nrb, b_proj, 0)

  wob_cp.wait()
  r128 = jax.lax.broadcasted_iota(jnp.int32, (128, 128), 0) // DH
  c128 = jax.lax.broadcasted_iota(jnp.int32, (128, 128), 1) // DH
  same_head = r128 == c128
  for g in range(G):
    blk = jnp.where(same_head, kv[g], 0.0).astype(BF16)
    mb[g * 128:(g + 1) * 128, :] = _dot(blk, wob[g * 128:(g + 1) * 128, :]).astype(BF16)

  def out_copy(src, col, i, sem):
    return pltpu.make_async_copy(
        src.at[pl.ds(i * RB, RB), :],
        out_hbm.at[pl.ds(i * RB, RB), pl.ds(col, D)],
        out_sem.at[sem])

  def b_out(i, carry):
    rows = pl.ds(pl.multiple_of(i * RB, RB), RB)
    parts = []
    for g in range(G):
      j, u = divmod(g, CB // 128)
      z = jnp.sum(zs[j, :, u * 128:(u + 1) * 128], axis=0, keepdims=True)
      zt = jnp.where(same_head, jnp.broadcast_to(z, (128, 128)), 0.0).astype(BF16)
      q = pq[rows, g * 128:(g + 1) * 128]
      den = _dot(q, zt, NT) + 1e-6
      parts.append((q.astype(F32) / den).astype(BF16))
    outb[rows, :] = _dot(jnp.concatenate(parts, axis=1), mb[...]).astype(BF16)
    for i_ in range(nrb):
      @pl.when(i == i_)
      def _():
        out_copy(outb, D, i_, i_).start()
    return carry

  jax.lax.fori_loop(0, nrb, b_out, 0)

  xa_cp.wait()
  wa_cp.wait()
  q_scale = DH ** -0.5 * math.log2(math.e)

  def a_proj(n, carry):
    j, i = n // nrb, n % nrb
    rows = pl.ds(pl.multiple_of(i * RB, RB), RB)
    x = xa[rows, :]

    def cols(p):
      return pl.ds(pl.multiple_of(p * D + j * CB, CB), CB)

    q = (_dot(x, wa[:, cols(0)]) * q_scale).T.astype(BF16)
    qt[i, cols(0), :] = q
    vt[cols(0), rows] = _dot(x, wa[:, cols(2)]).T.astype(BF16)
    k = _dot(x, wa[:, cols(1)]).astype(BF16)
    for u in range(CB // 128):
      kk[j * (CB // 128) + u, rows, :] = k[:, u * 128:(u + 1) * 128]
    return carry

  jax.lax.fori_loop(0, ncb * nrb, a_proj, 0)

  woa_cp.wait()
  s_buf, m_buf = (s0, s1), (m0, m1)
  head_of_row = jax.lax.broadcasted_iota(jnp.int32, (128, 1), 0) // DH
  st = {"mh": [], "lh": []}

  def scores(t, slot, c):
    qb, h = t // H, t % H
    g = h // 4
    if c == 0:
      q = qt[qb, pl.ds(pl.multiple_of(g * 128, 128), 128), :]
      st["q"] = jnp.where(head_of_row == h % 4, q, jnp.zeros_like(q))
      st["macc"] = None
    keys = slice(c * CK, (c + 1) * CK)
    s = _dot(kk[g, keys, :], st["q"])
    s_buf[slot][keys, :] = s
    macc = st["macc"]
    for r in range(CK // 8):
      sr = s[r * 8:(r + 1) * 8]
      macc = sr if macc is None else jnp.maximum(macc, sr)
    st["macc"] = macc
    st["mh"].append(macc)
    if c == NC - 1:
      m_buf[slot][...] = jnp.broadcast_to(
          jnp.max(macc, axis=0, keepdims=True), (8, TQ))

  def values(t, slot, c):
    qb, h = t // H, t % H
    if c == 0:
      st["lacc"], st["oacc"], st["lh"] = None, None, []
    m = m_buf[slot][...]
    if len(st["lh"]) >= 2:
      m = jnp.maximum(m, m - st["lh"][-2])
    if len(st["mh"]) >= 3:
      m = jnp.minimum(m, jnp.maximum(m, st["mh"][-3]))
    keys = slice(c * CK, (c + 1) * CK)
    p = jnp.exp2(s_buf[slot][keys, :].reshape(CK // 8, 8, TQ) - m[None])
    lacc = st["lacc"]
    for r in reversed(range(CK // 8)):
      lacc = p[r] if lacc is None else lacc + p[r]
    st["lacc"] = lacc
    st["lh"].append(lacc)
    v = vt[pl.ds(pl.multiple_of(h * DH, DH), DH), keys]
    oc = _dot(v, p.reshape(CK, TQ).astype(BF16))
    st["oacc"] = oc if st["oacc"] is None else st["oacc"] + oc
    if c == NC - 1:
      l = jnp.sum(lacc, axis=0, keepdims=True)
      ot[qb, pl.ds(pl.multiple_of(h * DH, DH), DH), :] = (st["oacc"] / l).astype(BF16)

  def step(t0, u, do_scores=True, do_tail=True, do_values=True):
    for c in range(NC):
      if do_scores:
        scores(t0 + u + 1, (u + 1) % 2, c)
      if c < LAG:
        if do_tail:
          values(t0 + u - 1, (u - 1) % 2, NC - LAG + c)
      elif do_values:
        values(t0 + u, u % 2, c - LAG)

  def project_out(qb):
    outa[pl.ds(pl.multiple_of(qb * TQ, TQ), TQ), :] = _dot(
        ot[qb], woa[...], TN).astype(BF16)

  nsteps = NQ * H
  nloop = (nsteps - 2) // UNROLL
  per_qb = H // UNROLL
  step(0, -1, True, False, False)
  step(0, 0, True, False, True)

  def attn(i, carry):
    st["lacc"], st["oacc"] = carry
    st["lh"], st["mh"] = [st["lacc"]], []
    for u in range(1, UNROLL + 1):
      step(UNROLL * i, u)

    @pl.when((i + 1) % per_qb == 0)
    def _():
      qb = (i + 1) // per_qb - 1
      project_out(qb)
      for qb_ in range(NQ - 1):
        @pl.when(qb == qb_)
        def _():
          out_copy(outa, 0, qb_, nrb + qb_).start()

    return st["lacc"], st["oacc"]

  st["lacc"], st["oacc"] = jax.lax.fori_loop(
      0, nloop, attn, (st["lacc"], st["oacc"]))
  st["lh"], st["mh"] = [st["lacc"]], []
  for u in range(nloop * UNROLL + 1, nsteps - 1):
    step(0, u)
  step(0, nsteps - 1, False, True, True)
  step(0, nsteps, False, True, False)
  project_out(NQ - 1)
  out_copy(outa, 0, NQ - 1, nrb + NQ - 1).start()

  for i_ in range(nrb):
    out_copy(outb, D, i_, i_).wait()
  for qb_ in range(NQ):
    out_copy(outa, 0, qb_, nrb + qb_).wait()


@jax.jit
def pallas_concat_heads__mha_block__linear_attn_block__prompt_kernel(
    A_x: jax.Array,
    A_wqkv: jax.Array,
    A_wo: jax.Array,
    B_x: jax.Array,
    B_wqkv: jax.Array,
    B_wo: jax.Array,
):
  assert A_x.shape == (1, S, D) and B_x.shape == (1, S, D)
  vmem = pltpu.VMEM
  any_spec = pl.BlockSpec(memory_space=pl.ANY)
  out = pl.pallas_call(
      _kernel,
      out_shape=jax.ShapeDtypeStruct((S, 2 * D), BF16),
      in_specs=[any_spec] * 6,
      out_specs=any_spec,
      scratch_shapes=[
          vmem((S, D), BF16), vmem((D, 3 * D), BF16), vmem((D, D), BF16),
          vmem((S, D), BF16), vmem((D, 3 * D), BF16), vmem((D, D), BF16),
          vmem((S, D), BF16),
          vmem((G, 128, 128), F32),
          vmem((D // CB, 8, CB), F32),
          vmem((D, D), BF16),
          vmem((S, D), BF16),
          vmem((NQ, D, TQ), BF16),
          vmem((G, S, 128), BF16),
          vmem((D, S), BF16),
          vmem((S, TQ), F32), vmem((S, TQ), F32),
          vmem((8, TQ), F32), vmem((8, TQ), F32),
          vmem((NQ, D, TQ), BF16),
          vmem((S, D), BF16),
          pltpu.SemaphoreType.DMA((16,)),
          pltpu.SemaphoreType.DMA((8,)),
      ],
      compiler_params=pltpu.CompilerParams(vmem_limit_bytes=100 * 2**20),
  )(A_x.reshape(S, D), A_wqkv, A_wo, B_x.reshape(S, D), B_wqkv, B_wo)
  return out.reshape(1, S, 2 * D)
```

```python
import math

import jax
import jax.numpy as jnp
import jax.experimental.pallas as pl
import jax.experimental.pallas.tpu as pltpu

S = 2048
D = 1024
H = 32
DH = D // H
G = D // 128

TQ = 512
CK = 128
NC = S // CK
NQ = S // TQ
LAG = 2
UNROLL = 4 * 2
PIECES = 4
AHEAD = 10

RB = 512
CB = 512
KR = 128
NRB = S // RB
NCB = D // CB

F32 = jnp.float32
BF16 = jnp.bfloat16
NN = (((1,), (0,)), ((), ()))
NT = (((1,), (1,)), ((), ()))


def _dot(a, b, dims=NN):
  return jax.lax.dot_general(a, b, dims, preferred_element_type=F32)


def _phi(t):
  return jnp.where(t > 0, t + 1.0, jnp.exp(t)) + 1e-6


def _ds(start, size):
  return pl.ds(pl.multiple_of(start, size), size)


def _iota(shape, axis):
  return jax.lax.broadcasted_iota(jnp.int32, shape, axis)


def _at_step(i, actions):
  for n, (wait, start) in actions.items():
    @pl.when(i == n)
    def _():
      for cp in wait:
        cp.wait()
      for cp in start:
        cp.start()


def _kernel(
    xa_hbm, wa_hbm, woa_hbm, xb_hbm, wb_hbm, wob_hbm, out_hbm,
    xa, wa, woa, xb, wb, wob,
    pkt, zs, zt, kv, mb, outb,
    qt, kk, vt, s0, s1, m0, m1, ot, oa, outa,
    in_sem, out_sem,
):
  def load(src, dst, sem, idx=(slice(None), slice(None))):
    return pltpu.make_async_copy(src.at[idx], dst.at[idx], in_sem.at[sem])

  def store(src, r0, c0, ncols, col_offset, sem):
    return pltpu.make_async_copy(
        src.at[pl.ds(r0, RB), pl.ds(c0, ncols)],
        out_hbm.at[pl.ds(r0, RB), pl.ds(col_offset + c0, ncols)],
        out_sem.at[sem])

  every = slice(None)
  x0_cp = [load(xb_hbm, xb, i, (pl.ds(i * (RB // 2), RB // 2), every))
           for i in range(2)]
  xb_cp = {i: load(xb_hbm, xb, 1 + i, (pl.ds(i * RB, RB), every))
           for i in range(1, NRB)}
  wk_cp = [load(wb_hbm, wb, 5 + j, (every, pl.ds(D + j * CB, CB)))
           for j in range(NCB)]
  wv_cp = load(wb_hbm, wb, 7, (every, pl.ds(2 * D, D)))
  wq_cp = load(wb_hbm, wb, 8, (every, pl.ds(0, D)))
  wob_cp = load(wob_hbm, wob, 9)
  xa_cp = load(xa_hbm, xa, 10)
  wa_cp = load(wa_hbm, wa, 11)
  woa_cp = load(woa_hbm, woa, 12)
  outb_cp = [store(outb, i * RB, 0, D, D, i) for i in range(NRB)]
  outa_cp = [store(outa, i * TQ, 0, D, 0, NRB + i) for i in range(NQ - 1)]
  last_cp = [store(outa, (NQ - 1) * TQ, j * CB, CB, 0, NRB + NQ - 1 + j)
             for j in range(NCB)]

  def b_keys(r0, nrows, j, first=False):
    z = None if first else zs[j]
    for r in range(0, nrows, KR):
      rows = _ds(r0 + r, KR)
      pk = _phi(_dot(xb[rows, :], wb[:, D + j * CB:D + (j + 1) * CB]))
      zr = jnp.sum(pk.reshape(KR // 8, 8, CB), axis=0)
      z = zr if z is None else z + zr
      pkt[j * CB:(j + 1) * CB, rows] = pk.T.astype(BF16)
    zs[j] = z

  x0_cp[0].start()
  wk_cp[0].start()
  x0_cp[0].wait()
  wk_cp[0].wait()
  x0_cp[1].start()
  wk_cp[1].start()
  b_keys(0, RB // 2, 0, first=True)
  x0_cp[1].wait()
  b_keys(RB // 2, RB // 2, 0)
  wk_cp[1].wait()
  xb_cp[1].start()
  b_keys(0, RB, 1, first=True)

  def b_keys_loop(i, carry):
    _at_step(i, {1: ([xb_cp[1]], [xb_cp[2], xb_cp[3]]),
                 2: ([xb_cp[2]], [wv_cp, wob_cp]),
                 3: ([xb_cp[3]], [wq_cp])})
    for j in range(NCB):
      b_keys(i * RB, RB, j)
    return carry

  jax.lax.fori_loop(1, NRB, b_keys_loop, 0)

  xa_cp.start()

  def b_kx_loop(i, carry):
    _at_step(i, {1: ([], [wa_cp]), 3: ([], [woa_cp])})
    rows = _ds(i * (D // 4), D // 4)
    mb[rows, :] = _dot(pkt[rows, :], xb[...]).astype(BF16)
    return carry

  jax.lax.fori_loop(0, 4, b_kx_loop, 0)

  wv_cp.wait()
  wq_cp.wait()
  wob_cp.wait()
  same_head = _iota((128, 128), 0) // DH == _iota((128, 128), 1) // DH
  head_lanes = _iota((16, 128), 0) % 4 == _iota((16, 128), 1) // DH
  for g in range(G):
    j, u = divmod(g, CB // 128)
    z = jnp.sum(zs[j, :, u * 128:(u + 1) * 128], axis=0, keepdims=True)
    zt[g] = jnp.where(head_lanes, jnp.broadcast_to(z, (16, 128)), 0.0).astype(BF16)
  for g in range(G):
    kv[g] = _dot(mb[g * 128:(g + 1) * 128, :],
                 wb[:, 2 * D + g * 128:2 * D + (g + 1) * 128])
  for g in range(G):
    rows = slice(g * 128, (g + 1) * 128)
    blk = jnp.where(same_head, kv[g], 0.0).astype(BF16)
    mb[rows, :] = _dot(blk, wob[rows, :]).astype(BF16)

  def b_out_loop(i, carry):
    def q_feat(r, n, j):
      return _phi(_dot(xb[_ds(i * RB + r, n), :],
                       wb[:, j * CB:(j + 1) * CB])).astype(BF16)

    def normalise(q, j):
      parts = []
      for u in range(CB // 128):
        qg = q[:, u * 128:(u + 1) * 128]
        den = _dot(zt[j * (CB // 128) + u], qg, NT)[0:8] + 1e-6
        inv = 1.0 / den
        inv = jnp.concatenate(
            [jnp.broadcast_to(inv[h:h + 1], (DH, RB)) for h in range(4)], axis=0).T
        parts.append((qg.astype(F32) * inv).astype(BF16))
      return jnp.concatenate(parts, axis=1)

    q0 = q_feat(0, RB, 0)
    q1a = q_feat(0, RB // 2, 1)
    n0 = normalise(q0, 0)
    q1b = q_feat(RB // 2, RB // 2, 1)
    lo = _dot(n0, mb[0:CB, 0:CB])
    n1 = normalise(jnp.concatenate([q1a, q1b], axis=0), 1)
    hi = _dot(n0, mb[0:CB, CB:D])
    rows = _ds(i * RB, RB)
    outb[rows, 0:CB] = (lo + _dot(n1, mb[CB:D, 0:CB])).astype(BF16)
    outb[rows, CB:D] = (hi + _dot(n1, mb[CB:D, CB:D])).astype(BF16)
    _at_step(i, {n: ([], [outb_cp[n]]) for n in range(NRB)})
    return carry

  jax.lax.fori_loop(0, NRB, b_out_loop, 0)

  xa_cp.wait()
  wa_cp.wait()
  q_scale = DH ** -0.5 * math.log2(math.e)

  def a_proj_loop(n, carry):
    j, i = n // NRB, n % NRB
    rows = _ds(i * RB, RB)
    x = xa[rows, :]

    def cols(p):
      return _ds(p * D + j * CB, CB)

    qt[i, cols(0), :] = (_dot(x, wa[:, cols(0)]) * q_scale).T.astype(BF16)
    vt[cols(0), rows] = _dot(x, wa[:, cols(2)]).T.astype(BF16)
    k = _dot(x, wa[:, cols(1)]).astype(BF16)
    for u in range(CB // 128):
      kk[j * (CB // 128) + u, rows, :] = k[:, u * 128:(u + 1) * 128]
    return carry

  jax.lax.fori_loop(0, NCB * NRB, a_proj_loop, 0)

  woa_cp.wait()
  s_buf, m_buf = (s0, s1), (m0, m1)
  head_of_row = _iota((128, 1), 0) // DH
  piece = CK // 8 // PIECES
  st = {"maxes": [], "sums": []}

  def block_and_group(g0, u):
    grp = g0 + u // 4
    return grp // G, grp % G

  def scores(g0, u, c):
    qb, g = block_and_group(g0, u)
    if c == 0:
      q = qt[qb, _ds(g * 128, 128), :]
      st["q"] = jnp.where(head_of_row == u % 4, q, jnp.zeros_like(q))
      st["macc"] = None
    keys = slice(c * CK, (c + 1) * CK)
    s = _dot(kk[g, keys, :], st["q"])
    s_buf[u % 2][keys, :] = s
    macc = st["macc"]
    for r in range(CK // 8):
      sr = s[r * 8:(r + 1) * 8]
      macc = sr if macc is None else jnp.maximum(macc, sr)
      if (r + 1) % piece == 0:
        st["maxes"].append(macc)
    st["macc"] = macc
    if c == NC - 1:
      m_buf[u % 2][...] = jnp.broadcast_to(
          jnp.max(macc, axis=0, keepdims=True), (8, TQ))

  def values(g0, u, c):
    qb, g = block_and_group(g0, u)
    if c == 0:
      st["lacc"], st["oacc"], st["sums"] = None, None, []
    m = m_buf[u % 2][...]
    if len(st["sums"]) >= 2:
      m = jnp.maximum(m, m - st["sums"][-2])
    keys = slice(c * CK, (c + 1) * CK)
    s = s_buf[u % 2][keys, :].reshape(CK // 8, 8, TQ)
    parts = [None] * PIECES
    for i in range(PIECES):
      mi = m
      if len(st["maxes"]) >= AHEAD - i:
        mi = jnp.minimum(m, jnp.maximum(m, st["maxes"][i - AHEAD]))
      k = PIECES - 1 - i
      parts[k] = jnp.exp2(s[k * piece:(k + 1) * piece] - mi[None])
    p = jnp.concatenate(parts, axis=0)
    lacc = st["lacc"]
    for r in reversed(range(CK // 8)):
      lacc = p[r] if lacc is None else lacc + p[r]
    st["lacc"] = lacc
    st["sums"].append(lacc)
    v = vt[_ds((g * 4 + u % 4) * DH, DH), keys]
    oc = _dot(v, p.reshape(CK, TQ).astype(BF16))
    st["oacc"] = oc if st["oacc"] is None else st["oacc"] + oc
    if c == NC - 1:
      l = jnp.sum(lacc, axis=0, keepdims=True)
      ot[(u % 4) * DH:(u % 4 + 1) * DH, :] = st["oacc"] / l
      if u % 4 == 3:
        oa[_ds(qb * TQ, TQ), _ds(g * 128, 128)] = ot[...].T.astype(BF16)

  def step(g0, u, do_scores=True, do_tail=True, do_values=True, fill=None):
    for c in range(NC):
      if do_scores:
        scores(g0, u + 1, c)
      if fill is not None:
        fill(c)
      if c < LAG:
        if do_tail:
          values(g0, u - 1, NC - LAG + c)
      elif do_values:
        values(g0, u, c - LAG)

  nsteps = NQ * H
  nloop = (nsteps - 2) // UNROLL
  per_qb = H // UNROLL
  step(0, -1, do_tail=False, do_values=False)
  step(0, 0, do_tail=False)

  def attn_loop(i, carry):
    st["lacc"], st["oacc"] = carry
    st["sums"], st["maxes"] = [st["lacc"]], []
    for u in range(1, UNROLL + 1):
      step((UNROLL // 4) * i, u)

    @pl.when(((i + 1) % per_qb == 0) & (i < (NQ - 2) * per_qb))
    def _():
      qb = (i + 1) // per_qb - 1
      rows = _ds(qb * TQ, TQ)
      outa[rows, :] = _dot(oa[rows, :], woa[...]).astype(BF16)
      _at_step(qb, {n: ([], [outa_cp[n]]) for n in range(NQ - 2)})

    return st["lacc"], st["oacc"]

  st["lacc"], st["oacc"] = jax.lax.fori_loop(
      0, nloop, attn_loop, (st["lacc"], st["oacc"]))
  st["sums"], st["maxes"] = [st["lacc"]], []
  for u in range(nloop * UNROLL + 1, nsteps - 1):
    step(0, u)

  def deferred_projection(c):
    if c % 4 == 0:
      r0 = (NQ - 2) * TQ + (c // 4) * 128
      outa[r0:r0 + 128, :] = _dot(oa[r0:r0 + 128, :], woa[...]).astype(BF16)

  step(0, nsteps - 1, do_scores=False, fill=deferred_projection)
  outa_cp[NQ - 2].start()
  step(0, nsteps, do_scores=False, do_values=False)
  rows = slice((NQ - 1) * TQ, NQ * TQ)
  for j in range(NCB):
    cols = slice(j * CB, (j + 1) * CB)
    outa[rows, cols] = _dot(oa[rows, :], woa[:, cols]).astype(BF16)
    last_cp[j].start()

  for cp in outb_cp + outa_cp + last_cp:
    cp.wait()


@jax.jit
def pallas_concat_heads__mha_block__linear_attn_block__prompt_kernel(
    A_x: jax.Array,
    A_wqkv: jax.Array,
    A_wo: jax.Array,
    B_x: jax.Array,
    B_wqkv: jax.Array,
    B_wo: jax.Array,
):
  assert A_x.shape == (1, S, D) and B_x.shape == (1, S, D)
  vmem = pltpu.VMEM
  any_spec = pl.BlockSpec(memory_space=pl.ANY)
  out = pl.pallas_call(
      _kernel,
      out_shape=jax.ShapeDtypeStruct((S, 2 * D), BF16),
      in_specs=[any_spec] * 6,
      out_specs=any_spec,
      scratch_shapes=[
          vmem((S, D), BF16), vmem((D, 3 * D), BF16), vmem((D, D), BF16),
          vmem((S, D), BF16), vmem((D, 3 * D), BF16), vmem((D, D), BF16),
          vmem((D, S), BF16),
          vmem((NCB, 8, CB), F32),
          vmem((G, 16, 128), BF16),
          vmem((G, 128, 128), F32),
          vmem((D, D), BF16),
          vmem((S, D), BF16),
          vmem((NQ, D, TQ), BF16),
          vmem((G, S, 128), BF16),
          vmem((D, S), BF16),
          vmem((S, TQ), F32), vmem((S, TQ), F32),
          vmem((8, TQ), F32), vmem((8, TQ), F32),
          vmem((128, TQ), F32),
          vmem((S, D), BF16),
          vmem((S, D), BF16),
          pltpu.SemaphoreType.DMA((13,)),
          pltpu.SemaphoreType.DMA((NRB + NQ - 1 + NCB,)),
      ],
      compiler_params=pltpu.CompilerParams(vmem_limit_bytes=100 * 2**20),
  )(A_x.reshape(S, D), A_wqkv, A_wo, B_x.reshape(S, D), B_wqkv, B_wo)
  return out.reshape(1, S, 2 * D)
```
